```python
import os as _os
_os.environ.setdefault("JAX_PLATFORMS", "cpu")
import jax
import jax.numpy as jnp

def _softmax(x, axis=-1):
    return jax.nn.softmax(x, axis=axis)
def _gelu(x):
    return jax.nn.gelu(x, approximate=True)
def _silu(x):
    return jax.nn.silu(x)
def _sigmoid(x):
    return jax.nn.sigmoid(x)
def _layernorm(x, axis=-1, eps=1e-5):
    m = jnp.mean(x, axis=axis, keepdims=True)
    v = jnp.var(x, axis=axis, keepdims=True)
    return (x - m) / jnp.sqrt(v + eps)
def _scatter_add(tgt, idx, src, axis=0):
    return tgt.at[idx].add(src)
def _segment_sum(src, seg, n):
    return jax.ops.segment_sum(src, seg, n)
class _Rng:
    def __init__(self, key):
        self._k = key
    def _next(self):
        self._k, sub = jax.random.split(self._k)
        return sub
    def normal(self, shape):
        return jax.random.normal(self._next(), shape, dtype=jnp.bfloat16)
    def randint(self, lo, hi, shape):
        return jax.random.randint(self._next(), shape, lo, hi, dtype=jnp.int32)
    def uniform(self, shape, lo=0.0, hi=1.0):
        return jax.random.uniform(self._next(), shape, jnp.bfloat16, lo, hi)
    def permutation(self, n):
        return jax.random.permutation(self._next(), n)


kernel_name = 'standalone__mha_softmax__near_ridge'

def setup_inputs():
    _rng = _Rng(jax.random.key(int.from_bytes(__import__("os").urandom(4), "little")))
    _w = (lambda a: (lambda t: t.astype(jnp.bfloat16) if jnp.issubdtype(t.dtype, jnp.floating) else t)(jnp.asarray(a)))
    B, H, Sq, Sk, D = 8, 32, 496, 512, 192
    return {
        "q": _w((lambda *s: _rng.normal(s) * 0.05)(B, H, Sq, D)),
        "k": _w((lambda *s: _rng.normal(s) * 3.2)(B, H, Sk, D)),
        "v": _w((lambda *s: _rng.normal(s) * 0.05)(B, H, Sk, D)),
    }

def reference(q, k, v):
    scale = q.shape[-1] ** -0.5
    scores = jnp.einsum("bhqd,bhkd->bhqk", q, k) * scale
    p = _softmax(scores, axis=-1)
    return jnp.einsum("bhqk,bhkd->bhqd", p, v)
```

```python
import functools

import jax
import jax.numpy as jnp
import jax.experimental.pallas as pl
import jax.experimental.pallas.tpu as pltpu

_LOG2E = 1.4426950408889634


def _scores(q_ref, k_ref, h):
    s = jax.lax.dot_general(k_ref[h], q_ref[h], (((0,), (0,)), ((), ())),
                            preferred_element_type=jnp.float32)
    return s, jnp.max(s, axis=0, keepdims=True)


def _attn_kernel(q_ref, k_ref, v_ref, o_ref, *, scale, heads):
    cur = _scores(q_ref, k_ref, 0)
    for h in range(heads):
        nxt = _scores(q_ref, k_ref, h + 1) if h + 1 < heads else None
        s_t, m = cur
        p_t = jnp.exp2((s_t - m) * (scale * _LOG2E))
        l = jnp.sum(p_t, axis=0, keepdims=True)
        o_t = jax.lax.dot_general(v_ref[h], p_t.astype(jnp.bfloat16),
                                  (((1,), (0,)), ((), ())),
                                  preferred_element_type=jnp.float32)
        o_ref[h] = (o_t / l).astype(o_ref.dtype)
        cur = nxt


@jax.jit
def pallas_standalone__mha_softmax__near_ridge_kernel(q, k, v):
    B, H, Sq, D = q.shape
    Sk = k.shape[2]
    BH = B * H
    heads = 8
    q_t = jnp.swapaxes(q, 2, 3).reshape(BH, D, Sq)
    k_t = jnp.swapaxes(k, 2, 3).reshape(BH, D, Sk)
    v_t = jnp.swapaxes(v, 2, 3).reshape(BH, D, Sk)
    scale = float(D) ** -0.5
    out = pl.pallas_call(
        functools.partial(_attn_kernel, scale=scale, heads=heads),
        grid=(BH // heads,),
        in_specs=[
            pl.BlockSpec((heads, D, Sq), lambda i: (i, 0, 0)),
            pl.BlockSpec((heads, D, Sk), lambda i: (i, 0, 0)),
            pl.BlockSpec((heads, D, Sk), lambda i: (i, 0, 0)),
        ],
        out_specs=pl.BlockSpec((heads, D, Sq), lambda i: (i, 0, 0)),
        out_shape=jax.ShapeDtypeStruct((BH, D, Sq), q.dtype),
        compiler_params=pltpu.CompilerParams(
            dimension_semantics=("parallel",),
            vmem_limit_bytes=64 * 1024 * 1024,
        ),
    )(q_t, k_t, v_t)
    return jnp.swapaxes(out.reshape(B, H, D, Sq), 2, 3)
```
